```python
import jax
import jax.numpy as jnp

def _softmax(x, axis=-1):
    return jax.nn.softmax(x, axis=axis)
def _gelu(x):
    return jax.nn.gelu(x, approximate=True)
def _silu(x):
    return jax.nn.silu(x)
def _sigmoid(x):
    return jax.nn.sigmoid(x)
def _layernorm(x, axis=-1, eps=1e-5):
    m = jnp.mean(x, axis=axis, keepdims=True)
    v = jnp.var(x, axis=axis, keepdims=True)
    return (x - m) / jnp.sqrt(v + eps)
def _scatter_add(tgt, idx, src, axis=0):
    return tgt.at[idx].add(src)
def _segment_sum(src, seg, n):
    return jax.ops.segment_sum(src, seg, n)
class _Rng:
    def __init__(self, key):
        self._k = key
    def _next(self):
        self._k, sub = jax.random.split(self._k)
        return sub
    def normal(self, shape):
        return jax.random.normal(self._next(), shape, dtype=jnp.bfloat16)
    def randint(self, lo, hi, shape):
        return jax.random.randint(self._next(), shape, lo, hi, dtype=jnp.int32)
    def uniform(self, shape, lo=0.0, hi=1.0):
        return jax.random.uniform(self._next(), shape, jnp.bfloat16, lo, hi)
    def permutation(self, n):
        return jax.random.permutation(self._next(), n)


kernel_name = 'parallel_sum__gqa_block_cached__moe_arch_mod__decode'

def setup_inputs():
    _rng = _Rng(jax.random.key(int.from_bytes(__import__("os").urandom(4), "little")))
    _w = (lambda a: (lambda t: t.astype(jnp.bfloat16) if jnp.issubdtype(t.dtype, jnp.floating) else t)(jnp.asarray(a)))
    def _A_setup():
        B, Sq, D = 1, 1, 448
        Hq, Hkv, Sk, Dh = 16, 8, 65536, 256
        assert Hq % Hkv == 0, (Hq, Hkv)
        return {
            "x": _w((lambda *s: _rng.normal(s) * 0.05)(B, Sq, D)),
            "k_cache": _w((lambda *s: _rng.normal(s) * 0.05)(B, Hkv, Sk, Dh)),
            "v_cache": _w((lambda *s: _rng.normal(s) * 0.05)(B, Hkv, Sk, Dh)),
            "wq": _w((lambda *s: _rng.normal(s) * 0.05)(D, Hq * Dh) * (D ** -0.5)),
            "wo": _w((lambda *s: _rng.normal(s) * 0.05)(Hq * Dh, D) * ((Hq * Dh) ** -0.5)),
        }
    _A_in = _A_setup()

    def _B_setup():
        B, S, D, F, C = 1, 1, 448, 1792, 1
        return {
            "x": _w((lambda *s: _rng.normal(s) * 0.05)(B, S, D)),
            "w_r": _w((lambda *s: _rng.normal(s) * 0.05)(D)),
            "w_gate": _w((lambda *s: _rng.normal(s) * 0.05)(D, F)),
            "w_up": _w((lambda *s: _rng.normal(s) * 0.05)(D, F)),
            "w_down": _w((lambda *s: _rng.normal(s) * 0.05)(F, D)),
        }
    _B_in = _B_setup()

    return {
        "A_x": _A_in["x"],
        "A_k_cache": _A_in["k_cache"],
        "A_v_cache": _A_in["v_cache"],
        "A_wq": _A_in["wq"],
        "A_wo": _A_in["wo"],
        "B_x": _B_in["x"],
        "B_w_r": _B_in["w_r"],
        "B_w_gate": _B_in["w_gate"],
        "B_w_up": _B_in["w_up"],
        "B_w_down": _B_in["w_down"],
    }

def reference(A_x, A_k_cache, A_v_cache, A_wq, A_wo, B_x, B_w_r, B_w_gate, B_w_up, B_w_down):
    def _A_ref(x, k_cache, v_cache, wq, wo):
        B, Sq, D = x.shape
        Hq, Dh = 16, 256
        Hkv = k_cache.shape[1]
        rep = Hq // Hkv
        q = (lambda x, *d: x.transpose(*d))((x @ wq).reshape(B, Sq, Hq, Dh), 0, 2, 1, 3)
        k = jnp.repeat(k_cache, rep, axis=1)
        v = jnp.repeat(v_cache, rep, axis=1)
        scores = jnp.einsum("bhqd,bhkd->bhqk", q, k) * (Dh ** -0.5)
        p = _softmax(scores, axis=-1)
        o = jnp.einsum("bhqk,bhkd->bhqd", p, v)
        return (lambda x, *d: x.transpose(*d))(o, 0, 2, 1, 3).reshape(B, Sq, Hq * Dh) @ wo

    def _B_ref(x, w_r, w_gate, w_up, w_down):
        B, S, D = x.shape
        C = 1
        r = x @ w_r
        idx = jnp.argsort(-r, axis=-1)[:, :C]
        idx_e = jnp.repeat(idx.reshape(B, C, 1), D, axis=2)
        x_sel = jnp.take_along_axis(x, idx_e, axis=1)
        g = _silu(x_sel @ w_gate)
        u = x_sel @ w_up
        y = (g * u) @ w_down
        r_sel = _sigmoid(jnp.take_along_axis(r, idx, axis=1))
        y = y * r_sel.reshape(B, C, 1)
        b_off = (jnp.arange(B) * S).reshape(B, 1)
        flat_idx = (idx + b_off).reshape(B * C)
        zero = (x * 0.0).reshape(B * S, D)
        upd = _scatter_add(zero, flat_idx, y.reshape(B * C, D), axis=0)
        return x + upd.reshape(B, S, D)

    x = A_x
    xn = _layernorm(x, axis=-1)
    return x + _A_ref(xn, A_k_cache, A_v_cache, A_wq, A_wo) + _B_ref(xn, B_w_r, B_w_gate, B_w_up, B_w_down)
```

```python
import functools
import jax
import jax.numpy as jnp
import numpy as np
from jax.experimental import pallas as pl
from jax.experimental.pallas import tpu as pltpu

def build(BS=1024, NBUF=4, SUB=64, W1D=True, D=448, HQ=16, HKV=8, SK=65536, DH=256, F=1792):
    NB = SK // BS
    T = HKV * NB
    REP = HQ // HKV
    f32, bf16 = jnp.float32, jnp.bfloat16
    NT = (((1,), (1,)), ((), ()))

    def kern(x_hbm, k_hbm, v_hbm, wq_hbm, wo_hbm, wr_hbm, wg_hbm, wu_hbm, wd_hbm, o_ref,
             kb, vb, x_v, wq_v, wo_v, wr_v, wg_v, wu_v, wd_v, q_s, kvsem, wsem):
        def kv_start(t, slot):
            base = pl.multiple_of(t * BS, BS)
            for s in range(BS // SUB):
                rows = pl.ds(base + s * SUB, SUB)
                pltpu.make_async_copy(k_hbm.at[rows], kb.at[slot, pl.ds(s * SUB, SUB)], kvsem.at[0, slot]).start(priority=0)
                pltpu.make_async_copy(v_hbm.at[rows], vb.at[slot, pl.ds(s * SUB, SUB)], kvsem.at[1, slot]).start(priority=1)

        def load2d(src, dst, sem, nl):
            n = src.shape[1]
            w = n // nl
            def b(i, _):
                r = pl.ds(pl.multiple_of(i * 16, 16), 16)
                for c in range(nl):
                    pltpu.make_async_copy(src.at[r, pl.ds(c * w, w)], dst.at[r, pl.ds(c * w, w)], sem).start(priority=c % 2)
                return 0
            jax.lax.fori_loop(0, src.shape[0] // 16, b, 0, unroll=True)

        def wait_all(v, sem):
            pltpu.make_async_copy(v, v, sem).wait()

        cx = pltpu.make_async_copy(x_hbm, x_v, wsem.at[0]); cx.start()
        cr = pltpu.make_async_copy(wr_hbm, wr_v, wsem.at[1]); cr.start(priority=1)
        load2d(wg_hbm, wg_v, wsem.at[2], 2)
        load2d(wu_hbm, wu_v, wsem.at[3], 2)
        load2d(wd_hbm, wd_v, wsem.at[4], 2)
        load2d(wq_hbm, wq_v, wsem.at[5], 4)
        for i in range(NBUF - 1):
            kv_start(i, i)
        for i in range(HQ):
            for r in range(D // 64):
                pltpu.make_async_copy(wo_hbm.at[pl.ds(r * 64, 64), pl.ds(i * DH, DH)],
                                      wo_v.at[i, pl.ds(r * 64, 64)], wsem.at[6]).start(priority=r % 2)

        cx.wait()
        x = x_v[...].astype(f32)
        mu = jnp.mean(x, axis=-1, keepdims=True)
        xc = x - mu
        var = jnp.mean(xc * xc, axis=-1, keepdims=True)
        xn = (xc * jax.lax.rsqrt(var + 1e-5)).astype(bf16)
        xn8 = jnp.broadcast_to(xn, (8, D))
        xnf = xn.astype(f32)
        cr.wait()
        wr = wr_v[...].reshape(1, D) if W1D else wr_v[...]
        r = jnp.sum(xnf * wr.astype(f32), axis=-1, keepdims=True)
        wait_all(wg_v, wsem.at[2])
        g = jnp.dot(xn8, wg_v[...], preferred_element_type=f32)
        wait_all(wu_v, wsem.at[3])
        u = jnp.dot(xn8, wu_v[...], preferred_element_type=f32)
        a = (g * jax.nn.sigmoid(g) * u).astype(bf16)
        wait_all(wd_v, wsem.at[4])
        y = jax.lax.dot_general(a, wd_v[...], NT, preferred_element_type=f32)[0:1]
        y = y * jax.nn.sigmoid(r)
        base = x + (xnf + (xnf * 0.0 + y))
        wait_all(wq_v, wsem.at[5])
        q = jnp.dot(xn8, wq_v[...], preferred_element_type=f32).astype(bf16)
        q = q * bf16(DH ** -0.5)
        row = jax.lax.broadcasted_iota(jnp.int32, (8, DH), 0)
        for h in range(HKV):
            qh = jnp.zeros((8, DH), bf16)
            for r_ in range(REP):
                c0 = (h * REP + r_) * DH
                qh = jnp.where(row == r_, q[:, c0:c0 + DH], qh)
            q_s[h] = qh
        wait_all(wo_v, wsem.at[6])

        def body(t, carry):
            m, l, acc, out = carry
            slot = t % NBUF
            h = t // NB
            j = t % NB
            nxt = t + (NBUF - 1)
            @pl.when(nxt < T)
            def _():
                kv_start(nxt, nxt % NBUF)
            wait_all(kb.at[slot], kvsem.at[0, slot])
            first = j == 0
            m = jnp.where(first, -jnp.inf, m)
            l = jnp.where(first, 0.0, l)
            acc = jnp.where(first, 0.0, acc)
            s = jax.lax.dot_general(q_s[h], kb[slot], NT, preferred_element_type=f32)
            m_new = jnp.maximum(m, jnp.max(s, axis=-1, keepdims=True))
            alpha = jnp.exp(m - m_new)
            p = jnp.exp(s - m_new)
            l = l * alpha + jnp.sum(p, axis=-1, keepdims=True)
            wait_all(vb.at[slot], kvsem.at[1, slot])
            acc = acc * alpha + jnp.dot(p.astype(bf16), vb[slot], preferred_element_type=f32)
            def fin(out):
                o = (acc / l).astype(bf16)
                for r_ in range(REP):
                    w = wo_v[h * REP + r_]
                    out = out + jax.lax.dot_general(o, w, NT, preferred_element_type=f32)[r_:r_ + 1]
                return out
            out = jax.lax.cond(j == NB - 1, fin, lambda o: o, out)
            return m_new, l, acc, out

        init = (jnp.full((8, 1), -jnp.inf, f32), jnp.zeros((8, 1), f32), jnp.zeros((8, DH), f32), jnp.zeros((1, D), f32))
        _, _, _, out = jax.lax.fori_loop(0, T, body, init)
        o_ref[...] = (base + out).astype(o_ref.dtype)

    hbm = pl.BlockSpec(memory_space=pltpu.HBM)
    call = pl.pallas_call(
        kern,
        out_shape=jax.ShapeDtypeStruct((1, D), bf16),
        in_specs=[hbm] * 9,
        out_specs=pl.BlockSpec(memory_space=pltpu.VMEM),
        scratch_shapes=[
            pltpu.VMEM((NBUF, BS, DH), bf16), pltpu.VMEM((NBUF, BS, DH), bf16),
            pltpu.VMEM((1, D), bf16), pltpu.VMEM((D, HQ * DH), bf16), pltpu.VMEM((HQ, D, DH), bf16),
            pltpu.VMEM((D,) if W1D else (1, D), bf16), pltpu.VMEM((D, F), bf16), pltpu.VMEM((D, F), bf16), pltpu.VMEM((D, F), bf16),
            pltpu.VMEM((HKV, 8, DH), bf16),
            pltpu.SemaphoreType.DMA((2, NBUF)), pltpu.SemaphoreType.DMA((7,)),
        ],
        compiler_params=pltpu.CompilerParams(vmem_limit_bytes=100 * 1024 * 1024),
    )

    @jax.jit
    def fn(A_x, A_k_cache, A_v_cache, A_wq, A_wo, B_x, B_w_r, B_w_gate, B_w_up, B_w_down):
        out = call(A_x.reshape(1, D), A_k_cache.reshape(HKV * SK, DH), A_v_cache.reshape(HKV * SK, DH),
                   A_wq, A_wo.T, B_w_r if W1D else B_w_r.reshape(1, D), B_w_gate, B_w_up, B_w_down.T)
        return out.reshape(1, 1, D)
    return fn


_kernel = build()


@jax.jit
def pallas_parallel_sum__gqa_block_cached__moe_arch_mod__decode_kernel(
    A_x: jax.Array,
    A_k_cache: jax.Array,
    A_v_cache: jax.Array,
    A_wq: jax.Array,
    A_wo: jax.Array,
    B_x: jax.Array,
    B_w_r: jax.Array,
    B_w_gate: jax.Array,
    B_w_up: jax.Array,
    B_w_down: jax.Array,
):
    return _kernel(A_x, A_k_cache, A_v_cache, A_wq, A_wo, B_x, B_w_r, B_w_gate, B_w_up, B_w_down)
```

```python
import jax
import jax.numpy as jnp
from jax.experimental import pallas as pl
from jax.experimental.pallas import tpu as pltpu

def build(BS=2048, NBUF=4, SUB=96, D=448, HQ=16, HKV=8, SK=65536, DH=256, F=1792):
    NB = SK // BS
    T = HKV * NB
    REP = HQ // HKV
    f32, bf16 = jnp.float32, jnp.bfloat16
    NT = (((1,), (1,)), ((), ()))

    def kern(x_hbm, k_hbm, v_hbm, wq_hbm, wo_hbm, wr_hbm, wg_hbm, wu_hbm, wd_hbm, o_ref,
             kb, vb, x_v, wq_v, wo_v, wr_v, wg_v, wu_v, wd_v, q_s, kvsem, wsem):
        def kv_start(t, slot):
            base = pl.multiple_of(t * BS, BS)
            for r0 in range(0, BS, SUB):
                n = min(SUB, BS - r0)
                rows = pl.ds(base + r0, n)
                pltpu.make_async_copy(k_hbm.at[rows], kb.at[slot, pl.ds(r0, n)], kvsem.at[0, slot]).start(priority=0)
                pltpu.make_async_copy(v_hbm.at[rows], vb.at[slot, pl.ds(r0, n)], kvsem.at[1, slot]).start(priority=1)

        def load_pair(A, B, nl):
            (sa, da, ma, ra), (sb, db, mb, rb) = A, B
            n = sa.shape[1]
            w = n // nl
            for i in range(len(ra)):
                for c in range(nl):
                    for p, (s_, d_, m_, r_) in enumerate((A, B)):
                        r = pl.ds(r_[i], 16)
                        pltpu.make_async_copy(s_.at[r, pl.ds(c * w, w)], d_.at[r, pl.ds(c * w, w)], m_).start(priority=p)

        def wait_all(v, sem):
            pltpu.make_async_copy(v, v, sem).wait()

        cx = pltpu.make_async_copy(x_hbm, x_v, wsem.at[0]); cx.start()
        cr = pltpu.make_async_copy(wr_hbm, wr_v, wsem.at[1]); cr.start(priority=1)
        rows = list(range(0, D, 16))
        load_pair((wg_hbm, wg_v, wsem.at[2], rows), (wu_hbm, wu_v, wsem.at[3], rows), 2)
        hf = len(rows) // 2
        load_pair((wd_hbm, wd_v, wsem.at[4], rows[:hf]), (wd_hbm, wd_v, wsem.at[4], rows[hf:]), 2)
        load_pair((wq_hbm, wq_v, wsem.at[5], rows), (wo_hbm, wo_v, wsem.at[6], rows), 4)
        for i in range(NBUF - 1):
            kv_start(i, i)

        cx.wait()
        x = x_v[...].astype(f32)
        mu = jnp.mean(x, axis=-1, keepdims=True)
        xc = x - mu
        var = jnp.mean(xc * xc, axis=-1, keepdims=True)
        xn = (xc * jax.lax.rsqrt(var + 1e-5)).astype(bf16)
        xn8 = jnp.broadcast_to(xn, (8, D))
        xnf = xn.astype(f32)
        cr.wait()
        wr = wr_v[...].reshape(1, D)
        r = jnp.sum(xnf * wr.astype(f32), axis=-1, keepdims=True)
        wait_all(wg_v, wsem.at[2])
        g = jnp.dot(xn8, wg_v[...], preferred_element_type=f32)
        wait_all(wu_v, wsem.at[3])
        u = jnp.dot(xn8, wu_v[...], preferred_element_type=f32)
        a = (g * jax.nn.sigmoid(g) * u).astype(bf16)
        wait_all(wd_v, wsem.at[4])
        y = jax.lax.dot_general(a, wd_v[...], NT, preferred_element_type=f32)[0:1]
        y = y * jax.nn.sigmoid(r)
        base = x + (xnf + (xnf * 0.0 + y))
        wait_all(wq_v, wsem.at[5])
        q = jnp.dot(xn8, wq_v[...], preferred_element_type=f32).astype(bf16)
        q = q * bf16(DH ** -0.5)
        row = jax.lax.broadcasted_iota(jnp.int32, (8, DH), 0)
        for h in range(HKV):
            qh = jnp.zeros((8, DH), bf16)
            for r_ in range(REP):
                c0 = (h * REP + r_) * DH
                qh = jnp.where(row == r_, q[:, c0:c0 + DH], qh)
            q_s[h] = qh
        wait_all(wo_v, wsem.at[6])

        def body(t, carry):
            m, l, acc, out = carry
            slot = t % NBUF
            h = t // NB
            j = t % NB
            nxt = t + (NBUF - 1)
            @pl.when(nxt < T)
            def _():
                kv_start(nxt, nxt % NBUF)
            wait_all(kb.at[slot], kvsem.at[0, slot])
            first = j == 0
            m = jnp.where(first, -jnp.inf, m)
            l = jnp.where(first, 0.0, l)
            acc = jnp.where(first, 0.0, acc)
            s = jax.lax.dot_general(q_s[h], kb[slot], NT, preferred_element_type=f32)
            m_new = jnp.maximum(m, jnp.max(s, axis=-1, keepdims=True))
            alpha = jnp.exp(m - m_new)
            p = jnp.exp(s - m_new)
            l = l * alpha + jnp.sum(p, axis=-1, keepdims=True)
            wait_all(vb.at[slot], kvsem.at[1, slot])
            acc = acc * alpha + jnp.dot(p.astype(bf16), vb[slot], preferred_element_type=f32)
            def fin(out):
                o = (acc / l).astype(bf16)
                for r_ in range(REP):
                    w = wo_v[:, pl.ds(pl.multiple_of((h * REP + r_) * DH, DH), DH)]
                    out = out + jax.lax.dot_general(o, w, NT, preferred_element_type=f32)[r_:r_ + 1]
                return out
            out = jax.lax.cond(j == NB - 1, fin, lambda o: o, out)
            return m_new, l, acc, out

        init = (jnp.full((8, 1), -jnp.inf, f32), jnp.zeros((8, 1), f32), jnp.zeros((8, DH), f32), jnp.zeros((1, D), f32))
        _, _, _, out = jax.lax.fori_loop(0, T, body, init)
        o_ref[...] = (base + out).astype(o_ref.dtype)

    hbm = pl.BlockSpec(memory_space=pltpu.HBM)
    call = pl.pallas_call(
        kern,
        out_shape=jax.ShapeDtypeStruct((1, D), bf16),
        in_specs=[hbm] * 9,
        out_specs=pl.BlockSpec(memory_space=pltpu.VMEM),
        scratch_shapes=[
            pltpu.VMEM((NBUF, BS, DH), bf16), pltpu.VMEM((NBUF, BS, DH), bf16),
            pltpu.VMEM((1, D), bf16), pltpu.VMEM((D, HQ * DH), bf16), pltpu.VMEM((D, HQ * DH), bf16),
            pltpu.VMEM((D,), bf16), pltpu.VMEM((D, F), bf16), pltpu.VMEM((D, F), bf16), pltpu.VMEM((D, F), bf16),
            pltpu.VMEM((HKV, 8, DH), bf16),
            pltpu.SemaphoreType.DMA((2, NBUF)), pltpu.SemaphoreType.DMA((7,)),
        ],
        compiler_params=pltpu.CompilerParams(vmem_limit_bytes=100 * 1024 * 1024),
    )

    @jax.jit
    def fn(A_x, A_k_cache, A_v_cache, A_wq, A_wo, B_x, B_w_r, B_w_gate, B_w_up, B_w_down):
        out = call(A_x.reshape(1, D), A_k_cache.reshape(HKV * SK, DH), A_v_cache.reshape(HKV * SK, DH),
                   A_wq, A_wo.T, B_w_r, B_w_gate, B_w_up, B_w_down.T)
        return out.reshape(1, 1, D)
    return fn


_kernel = build()


@jax.jit
def pallas_parallel_sum__gqa_block_cached__moe_arch_mod__decode_kernel(
    A_x: jax.Array,
    A_k_cache: jax.Array,
    A_v_cache: jax.Array,
    A_wq: jax.Array,
    A_wo: jax.Array,
    B_x: jax.Array,
    B_w_r: jax.Array,
    B_w_gate: jax.Array,
    B_w_up: jax.Array,
    B_w_down: jax.Array,
):
    return _kernel(A_x, A_k_cache, A_v_cache, A_wq, A_wo, B_x, B_w_r, B_w_gate, B_w_up, B_w_down)
```

```python
import jax
import jax.numpy as jnp
from jax.experimental import pallas as pl
from jax.experimental.pallas import tpu as pltpu

BS = 2048
NBUF = 4
SUB = 96


@jax.jit
def pallas_parallel_sum__gqa_block_cached__moe_arch_mod__decode_kernel(
    A_x: jax.Array,
    A_k_cache: jax.Array,
    A_v_cache: jax.Array,
    A_wq: jax.Array,
    A_wo: jax.Array,
    B_x: jax.Array,
    B_w_r: jax.Array,
    B_w_gate: jax.Array,
    B_w_up: jax.Array,
    B_w_down: jax.Array,
):
    del B_x
    D, F = B_w_gate.shape
    _, HKV, SK, DH = A_k_cache.shape
    HQ = A_wq.shape[1] // DH
    assert A_x.shape == (1, 1, D) and SK % BS == 0 and D % 32 == 0
    NB = SK // BS
    T = HKV * NB
    REP = HQ // HKV
    f32, bf16 = jnp.float32, jnp.bfloat16
    NT = (((1,), (1,)), ((), ()))

    def kern(x_hbm, k_hbm, v_hbm, wq_hbm, wo_hbm, wr_hbm, wg_hbm, wu_hbm, wd_hbm, o_ref,
             kb, vb, x_v, wq_v, wo_v, wr_v, wg_v, wu_v, wd_v, q_s, kvsem, wsem):
        def kv_start(t, slot):
            base = pl.multiple_of(t * BS, BS)
            for r0 in range(0, BS, SUB):
                n = min(SUB, BS - r0)
                rows = pl.ds(base + r0, n)
                pltpu.make_async_copy(k_hbm.at[rows], kb.at[slot, pl.ds(r0, n)], kvsem.at[0, slot]).start(priority=0)
                pltpu.make_async_copy(v_hbm.at[rows], vb.at[slot, pl.ds(r0, n)], kvsem.at[1, slot]).start(priority=1)

        def load_pair(A, B, nl):
            (sa, da, ma, ra), (sb, db, mb, rb) = A, B
            n = sa.shape[1]
            w = n // nl
            for i in range(len(ra)):
                for c in range(nl):
                    for p, (s_, d_, m_, r_) in enumerate((A, B)):
                        r = pl.ds(r_[i], 16)
                        pltpu.make_async_copy(s_.at[r, pl.ds(c * w, w)], d_.at[r, pl.ds(c * w, w)], m_).start(priority=p)

        def wait_all(v, sem):
            pltpu.make_async_copy(v, v, sem).wait()

        cx = pltpu.make_async_copy(x_hbm, x_v, wsem.at[0]); cx.start()
        cr = pltpu.make_async_copy(wr_hbm, wr_v, wsem.at[1]); cr.start(priority=1)
        rows = list(range(0, D, 16))
        load_pair((wg_hbm, wg_v, wsem.at[2], rows), (wu_hbm, wu_v, wsem.at[3], rows), 2)
        hf = len(rows) // 2
        load_pair((wd_hbm, wd_v, wsem.at[4], rows[:hf]), (wd_hbm, wd_v, wsem.at[4], rows[hf:]), 2)
        load_pair((wq_hbm, wq_v, wsem.at[5], rows), (wo_hbm, wo_v, wsem.at[6], rows), 4)
        for i in range(NBUF - 1):
            kv_start(i, i)

        cx.wait()
        x = x_v[...].astype(f32)
        mu = jnp.mean(x, axis=-1, keepdims=True)
        xc = x - mu
        var = jnp.mean(xc * xc, axis=-1, keepdims=True)
        xn = (xc * jax.lax.rsqrt(var + 1e-5)).astype(bf16)
        xn8 = jnp.broadcast_to(xn, (8, D))
        xnf = xn.astype(f32)
        cr.wait()
        wr = wr_v[...].reshape(1, D)
        r = jnp.sum(xnf * wr.astype(f32), axis=-1, keepdims=True)
        wait_all(wg_v, wsem.at[2])
        g = jnp.dot(xn8, wg_v[...], preferred_element_type=f32)
        wait_all(wu_v, wsem.at[3])
        u = jnp.dot(xn8, wu_v[...], preferred_element_type=f32)
        a = (g * jax.nn.sigmoid(g) * u).astype(bf16)
        wait_all(wd_v, wsem.at[4])
        y = jax.lax.dot_general(a, wd_v[...], NT, preferred_element_type=f32)[0:1]
        y = y * jax.nn.sigmoid(r)
        base = x + (xnf + (xnf * 0.0 + y))
        wait_all(wq_v, wsem.at[5])
        q = jnp.dot(xn8, wq_v[...], preferred_element_type=f32).astype(bf16)
        q = q * bf16(DH ** -0.5)
        row = jax.lax.broadcasted_iota(jnp.int32, (8, DH), 0)
        for h in range(HKV):
            qh = jnp.zeros((8, DH), bf16)
            for r_ in range(REP):
                c0 = (h * REP + r_) * DH
                qh = jnp.where(row == r_, q[:, c0:c0 + DH], qh)
            q_s[h] = qh
        wait_all(wo_v, wsem.at[6])

        def body(t, carry):
            m, l, acc, out = carry
            slot = t % NBUF
            h = t // NB
            j = t % NB
            nxt = t + (NBUF - 1)
            @pl.when(nxt < T)
            def _():
                kv_start(nxt, nxt % NBUF)
            wait_all(kb.at[slot], kvsem.at[0, slot])
            first = j == 0
            m = jnp.where(first, -jnp.inf, m)
            l = jnp.where(first, 0.0, l)
            acc = jnp.where(first, 0.0, acc)
            s = jax.lax.dot_general(q_s[h], kb[slot], NT, preferred_element_type=f32)
            m_new = jnp.maximum(m, jnp.max(s, axis=-1, keepdims=True))
            alpha = jnp.exp(m - m_new)
            p = jnp.exp(s - m_new)
            l = l * alpha + jnp.sum(p, axis=-1, keepdims=True)
            wait_all(vb.at[slot], kvsem.at[1, slot])
            acc = acc * alpha + jnp.dot(p.astype(bf16), vb[slot], preferred_element_type=f32)
            def fin(out):
                o = (acc / l).astype(bf16)
                for r_ in range(REP):
                    w = wo_v[:, pl.ds(pl.multiple_of((h * REP + r_) * DH, DH), DH)]
                    out = out + jax.lax.dot_general(o, w, NT, preferred_element_type=f32)[r_:r_ + 1]
                return out
            out = jax.lax.cond(j == NB - 1, fin, lambda o: o, out)
            return m_new, l, acc, out

        init = (jnp.full((8, 1), -jnp.inf, f32), jnp.zeros((8, 1), f32), jnp.zeros((8, DH), f32), jnp.zeros((1, D), f32))
        _, _, _, out = jax.lax.fori_loop(0, T, body, init)
        o_ref[...] = (base + out).astype(o_ref.dtype)

    hbm = pl.BlockSpec(memory_space=pltpu.HBM)
    call = pl.pallas_call(
        kern,
        out_shape=jax.ShapeDtypeStruct((1, D), bf16),
        in_specs=[hbm] * 9,
        out_specs=pl.BlockSpec(memory_space=pltpu.VMEM),
        scratch_shapes=[
            pltpu.VMEM((NBUF, BS, DH), bf16), pltpu.VMEM((NBUF, BS, DH), bf16),
            pltpu.VMEM((1, D), bf16), pltpu.VMEM((D, HQ * DH), bf16), pltpu.VMEM((D, HQ * DH), bf16),
            pltpu.VMEM((D,), bf16), pltpu.VMEM((D, F), bf16), pltpu.VMEM((D, F), bf16), pltpu.VMEM((D, F), bf16),
            pltpu.VMEM((HKV, 8, DH), bf16),
            pltpu.SemaphoreType.DMA((2, NBUF)), pltpu.SemaphoreType.DMA((7,)),
        ],
        compiler_params=pltpu.CompilerParams(vmem_limit_bytes=100 * 1024 * 1024),
    )

    out = call(A_x.reshape(1, D), A_k_cache.reshape(HKV * SK, DH), A_v_cache.reshape(HKV * SK, DH),
               A_wq, A_wo.T, B_w_r, B_w_gate, B_w_up, B_w_down.T)
    return out.reshape(1, 1, D)
```
